```python
import os as _os
_os.environ.setdefault("JAX_PLATFORMS", "cpu")
import jax
import jax.numpy as jnp

def _softmax(x, axis=-1):
    return jax.nn.softmax(x, axis=axis)
def _gelu(x):
    return jax.nn.gelu(x, approximate=True)
def _silu(x):
    return jax.nn.silu(x)
def _sigmoid(x):
    return jax.nn.sigmoid(x)
def _layernorm(x, axis=-1, eps=1e-5):
    m = jnp.mean(x, axis=axis, keepdims=True)
    v = jnp.var(x, axis=axis, keepdims=True)
    return (x - m) / jnp.sqrt(v + eps)
def _scatter_add(tgt, idx, src, axis=0):
    return tgt.at[idx].add(src)
def _segment_sum(src, seg, n):
    return jax.ops.segment_sum(src, seg, n)
class _Rng:
    def __init__(self, key):
        self._k = key
    def _next(self):
        self._k, sub = jax.random.split(self._k)
        return sub
    def normal(self, shape):
        return jax.random.normal(self._next(), shape, dtype=jnp.bfloat16)
    def randint(self, lo, hi, shape):
        return jax.random.randint(self._next(), shape, lo, hi, dtype=jnp.int32)
    def uniform(self, shape, lo=0.0, hi=1.0):
        return jax.random.uniform(self._next(), shape, jnp.bfloat16, lo, hi)
    def permutation(self, n):
        return jax.random.permutation(self._next(), n)


kernel_name = 'standalone__channel_attn_cbam__vision'

def setup_inputs():
    _rng = _Rng(jax.random.key(int.from_bytes(__import__("os").urandom(4), "little")))
    _w = (lambda a: (lambda t: t.astype(jnp.bfloat16) if jnp.issubdtype(t.dtype, jnp.floating) else t)(jnp.asarray(a)))
    H = W = 224
    C = 192
    r = max(C // 4, 1)
    return {
        "x": _w((lambda *s: _rng.normal(s) * 0.2)(1, H, W, C) + (lambda *s: _rng.normal(s) * 0.2)(1, 1, 1, C) * 2.0),
        "w1": _w((lambda *s: _rng.normal(s) * 0.2)(C, r)),
        "w2": _w((lambda *s: _rng.normal(s) * 0.2)(r, C)),
    }

def reference(x, w1, w2):
    B, H, W, C = x.shape
    xf = x.reshape(B, H * W, C)
    gap = jnp.mean(xf, 1)
    gmp = jnp.amax(xf, 1)
    h_a = gap @ w1
    h_a = h_a * (lambda x, dt: x.astype(dt))(h_a > 0, h_a.dtype)
    h_m = gmp @ w1
    h_m = h_m * (lambda x, dt: x.astype(dt))(h_m > 0, h_m.dtype)
    scale = _sigmoid(h_a @ w2 + h_m @ w2)
    return x * scale[:, None, None, :]
```

```python
import jax
import jax.numpy as jnp
from jax import lax
import jax.experimental.pallas as pl
import jax.experimental.pallas.tpu as pltpu

NREG = 7
P0 = 1
CB = 16
T = 4
NS = 4
F = 3


def _bf16_round(v):
  return v.astype(jnp.bfloat16).astype(jnp.float32)


def _cbam_kernel(x_hbm, w1t_hbm, w2_hbm, o_hbm,
                 buf, w1t_v, w2_v, w1_s, w2t_s, acc_s, acc_m, scale_s, sem):
  _, J, C, W = buf.shape
  R = w1t_v.shape[0]
  NCB = C // CB
  AHEAD = NS - 1
  JM = J - T
  UC = NCB // T
  last_cb = (T - 1) * UC
  assert C % (CB * T) == 0 and UC == T - 1 == NS - 1 and JM >= NS

  def rows_of(cb, n=1):
    start = cb * CB
    if not isinstance(cb, int):
      start = pl.multiple_of(start, CB)
    return pl.ds(start, n * CB)

  def start_step(j, cb, s):
    for priority, regions in enumerate((pl.ds(0, P0), pl.ds(P0, NREG - P0))):
      idx = (regions, j, rows_of(cb), slice(None))
      pltpu.make_async_copy(x_hbm.at[idx], buf.at[idx], s).start(
          priority=priority)

  def wait_block(js, rows, s):
    idx = (slice(None), js, rows, slice(None))
    pltpu.make_async_copy(x_hbm.at[idx], buf.at[idx], s).wait()

  def start_main(u):
    for cb in range(NCB):
      start_step(u, cb, sem.at[u % NS])

  w1_cp = pltpu.make_async_copy(w1t_hbm, w1t_v, sem.at[0])
  w2_cp = pltpu.make_async_copy(w2_hbm, w2_v, sem.at[0])
  for u in range(AHEAD):
    start_main(u)
  w1_cp.start()
  w2_cp.start()

  acc_s[...] = jnp.zeros(acc_s.shape, jnp.float32)
  acc_m[...] = jnp.full(acc_m.shape, -jnp.inf, jnp.float32)

  def pooled(js, rows):
    s = acc_s[rows, :]
    m = acc_m[rows, :]
    for j in js:
      for k in range(NREG):
        v = buf[k, j, rows, :].astype(jnp.float32)
        s = s + v
        m = jnp.maximum(m, v)
    return s, m

  def accumulate(js, cb):
    rows = rows_of(cb)
    s, m = pooled(js, rows)
    acc_s[rows, :] = s
    acc_m[rows, :] = m

  def read_body(u, carry):
    nxt = u + AHEAD

    @pl.when(nxt < JM)
    def _():
      start_main(nxt)

    @pl.when(nxt >= JM)
    def _():
      for j in range(JM, J):
        for i in range(UC):
          start_step(j, (nxt - JM) * UC + i, sem.at[nxt % NS])

    wait_block(u, slice(None), sem.at[u % NS])

    @pl.when(u == 0)
    def _():
      w1_cp.wait()
      w2_cp.wait()
      w1_s[...] = w1t_v[...].astype(jnp.float32).T
      w2t_s[...] = w2_v[...].astype(jnp.float32).T

    for cb in range(NCB):
      accumulate([u], cb)
    return carry

  lax.fori_loop(0, JM, read_body, 0)

  inv_n = 1.0 / (NREG * J * W)

  def fold(js, cb, h):
    ha, hm = h
    rows = rows_of(cb)
    s, m = pooled(js, rows)
    gap = _bf16_round(jnp.sum(s, axis=1, keepdims=True) * inv_n)
    gmp = jnp.max(m, axis=1, keepdims=True)
    w = w1_s[rows, :]
    return ha + gap * w, hm + gmp * w

  def tail_body(t, h):
    part_sem = sem.at[(JM - 1 + t) % NS]
    for j in range(JM, J):
      start_step(j, last_cb + t, part_sem)
    wait_block(pl.ds(JM, T), rows_of(t * UC, UC), sem.at[(JM + t) % NS])
    for i in range(UC):
      h = fold(range(JM, J), t * UC + i, h)
    return h

  zero = jnp.zeros((CB, R), jnp.float32)
  h = lax.fori_loop(0, T - 1, tail_body, (zero, zero))

  for i in range(UC):
    wait_block(pl.ds(JM, T), rows_of(last_cb + i), sem.at[(JM - 1 + i) % NS])
    if i < UC - 1:
      accumulate(range(JM, J), last_cb + i)
  h = fold(range(JM, J), NCB - 1, h)
  for i in range(UC - 1):
    h = fold([], last_cb + i, h)
  ha, hm = h
  ha = _bf16_round(jnp.sum(ha, axis=0, keepdims=True))
  hm = _bf16_round(jnp.sum(hm, axis=0, keepdims=True))
  ha = ha * (ha > 0).astype(jnp.float32)
  hm = hm * (hm > 0).astype(jnp.float32)

  def gate(cb):
    rows = rows_of(cb)
    w = w2t_s[rows, :]
    za = _bf16_round(jnp.sum(w * ha, axis=1, keepdims=True))
    zm = _bf16_round(jnp.sum(w * hm, axis=1, keepdims=True))
    z = _bf16_round(za + zm)
    sc = _bf16_round(1.0 / (1.0 + jnp.exp(-z)))
    scale_s[rows, :] = jnp.broadcast_to(sc, (CB, W))

  def scale_and_send(j, cb):
    rows = rows_of(cb)
    sc = scale_s[rows, :]
    for k in range(NREG):
      v = buf[k, j, rows, :].astype(jnp.float32)
      buf[k, j, rows, :] = (v * sc).astype(buf.dtype)
    idx = (slice(None), j, rows, slice(None))
    pltpu.make_async_copy(buf.at[idx], o_hbm.at[idx], sem.at[0]).start()

  def first_row(cb, carry):
    scale_and_send(0, cb)
    return carry

  for cb in range(F):
    gate(cb)
  lax.fori_loop(0, F, first_row, 0)
  for cb in range(F, NCB):
    gate(cb)
  lax.fori_loop(F, NCB, first_row, 0)

  def write_body(j, carry):
    for cb in range(NCB):
      scale_and_send(j, cb)
    return carry

  lax.fori_loop(1, J, write_body, 0)
  pltpu.make_async_copy(buf, o_hbm, sem.at[0]).wait()


@jax.jit
def pallas_standalone__channel_attn_cbam__vision_kernel(
    x: jax.Array,
    w1: jax.Array,
    w2: jax.Array,
):
  B, H, W, C = x.shape
  R = w1.shape[1]
  assert B == 1 and H % NREG == 0
  shape = (NREG, H // NREG, C, W)
  out = pl.pallas_call(
      _cbam_kernel,
      in_specs=[pl.BlockSpec(memory_space=pl.ANY)] * 3,
      out_specs=pl.BlockSpec(memory_space=pl.ANY),
      out_shape=jax.ShapeDtypeStruct(shape, x.dtype),
      scratch_shapes=[
          pltpu.VMEM(shape, x.dtype),
          pltpu.VMEM((R, C), w1.dtype),
          pltpu.VMEM((R, C), w2.dtype),
          pltpu.VMEM((C, R), jnp.float32),
          pltpu.VMEM((C, R), jnp.float32),
          pltpu.VMEM((C, W), jnp.float32),
          pltpu.VMEM((C, W), jnp.float32),
          pltpu.VMEM((C, W), jnp.float32),
          pltpu.SemaphoreType.DMA((NS,)),
      ],
      compiler_params=pltpu.CompilerParams(vmem_limit_bytes=64 * 1024 * 1024),
  )(x.transpose(0, 1, 3, 2).reshape(shape), w1.T, w2)
  return out.reshape(B, H, C, W).transpose(0, 1, 3, 2)
```

```python
import jax
import jax.numpy as jnp
from jax import lax
import jax.experimental.pallas as pl
import jax.experimental.pallas.tpu as pltpu

NREG = 7
P0 = 1
CB = 16
T = 4
NS = 4
F = 3


def _bf16_round(v):
  return v.astype(jnp.bfloat16).astype(jnp.float32)


def _cbam_kernel(x_hbm, w1t_hbm, w2_hbm, o_hbm,
                 buf, w1t_v, w2_v, w1_s, w2t_s, acc_s, acc_m, scale_s, sem):
  _, J, C, W = buf.shape
  R = w1t_v.shape[0]
  NCB = C // CB
  AHEAD = NS - 1
  JM = J - T
  UC = NCB // T
  last_cb = (T - 1) * UC
  assert C % (CB * T) == 0 and UC == T - 1 == NS - 1 and JM >= NS

  def rows_of(cb, n=1):
    start = cb * CB
    if not isinstance(cb, int):
      start = pl.multiple_of(start, CB)
    return pl.ds(start, n * CB)

  def start_step(j, cb, s):
    for priority, regions in enumerate((pl.ds(0, P0), pl.ds(P0, NREG - P0))):
      idx = (regions, j, rows_of(cb), slice(None))
      pltpu.make_async_copy(x_hbm.at[idx], buf.at[idx], s).start(
          priority=priority)

  def wait_block(js, rows, s):
    idx = (slice(None), js, rows, slice(None))
    pltpu.make_async_copy(x_hbm.at[idx], buf.at[idx], s).wait()

  def start_main(u):
    for cb in range(NCB):
      start_step(u, cb, sem.at[u % NS])

  w1_cp = pltpu.make_async_copy(w1t_hbm, w1t_v, sem.at[AHEAD])
  w2_cp = pltpu.make_async_copy(w2_hbm, w2_v, sem.at[AHEAD])
  w1_cp.start()
  w2_cp.start()
  for u in range(AHEAD):
    start_main(u)

  acc_s[...] = jnp.zeros(acc_s.shape, jnp.float32)
  acc_m[...] = jnp.full(acc_m.shape, -jnp.inf, jnp.float32)
  w1_cp.wait()
  w2_cp.wait()
  w1_s[...] = w1t_v[...].astype(jnp.float32).T
  w2t_s[...] = w2_v[...].astype(jnp.float32).T

  def pooled(js, rows):
    s = acc_s[rows, :]
    m = acc_m[rows, :]
    for j in js:
      for k in range(NREG):
        v = buf[k, j, rows, :].astype(jnp.float32)
        s = s + v
        m = jnp.maximum(m, v)
    return s, m

  def accumulate(js, cb):
    rows = rows_of(cb)
    s, m = pooled(js, rows)
    acc_s[rows, :] = s
    acc_m[rows, :] = m

  def read_body(u, carry):
    nxt = u + AHEAD

    @pl.when(nxt < JM)
    def _():
      start_main(nxt)

    @pl.when(nxt >= JM)
    def _():
      for j in range(JM, J):
        for i in range(UC):
          start_step(j, (nxt - JM) * UC + i, sem.at[nxt % NS])

    wait_block(u, slice(None), sem.at[u % NS])
    for cb in range(NCB):
      accumulate([u], cb)
    return carry

  lax.fori_loop(0, JM, read_body, 0)

  inv_n = 1.0 / (NREG * J * W)

  def fold(js, cb, h):
    ha, hm = h
    rows = rows_of(cb)
    s, m = pooled(js, rows)
    gap = _bf16_round(jnp.sum(s, axis=1, keepdims=True) * inv_n)
    gmp = jnp.max(m, axis=1, keepdims=True)
    w = w1_s[rows, :]
    return ha + gap * w, hm + gmp * w

  final_sem = sem.at[(JM + UC - 1) % NS]

  def tail_body(t, h):
    part_sem = sem.at[(JM - 1 + t) % NS]
    for j in range(JM, J - 1):
      start_step(j, last_cb + t, part_sem)

    @pl.when(t < UC - 1)
    def _():
      start_step(J - 1, last_cb + t, part_sem)

    wait_block(pl.ds(JM, T), rows_of(t * UC, UC), sem.at[(JM + t) % NS])

    @pl.when(t == UC - 1)
    def _():
      start_step(J - 1, NCB - 1, final_sem)

    for i in range(UC):
      h = fold(range(JM, J), t * UC + i, h)
    return h

  zero = jnp.zeros((CB, R), jnp.float32)
  h = lax.fori_loop(0, T - 1, tail_body, (zero, zero))

  for i in range(UC):
    n = T if i < UC - 1 else T - 1
    wait_block(pl.ds(JM, n), rows_of(last_cb + i), sem.at[(JM - 1 + i) % NS])
    accumulate(range(JM, JM + n), last_cb + i)
  wait_block(J - 1, rows_of(NCB - 1), final_sem)
  h = fold([J - 1], NCB - 1, h)
  for i in range(UC - 1):
    h = fold([], last_cb + i, h)
  ha, hm = h
  ha = _bf16_round(jnp.sum(ha, axis=0, keepdims=True))
  hm = _bf16_round(jnp.sum(hm, axis=0, keepdims=True))
  ha = ha * (ha > 0).astype(jnp.float32)
  hm = hm * (hm > 0).astype(jnp.float32)

  def gate(cb):
    rows = rows_of(cb)
    w = w2t_s[rows, :]
    za = _bf16_round(jnp.sum(w * ha, axis=1, keepdims=True))
    zm = _bf16_round(jnp.sum(w * hm, axis=1, keepdims=True))
    sc = _bf16_round(jax.nn.sigmoid(_bf16_round(za + zm)))
    scale_s[rows, :] = jnp.broadcast_to(sc, (CB, W))

  def scale_and_send(j, cb):
    rows = rows_of(cb)
    sc = scale_s[rows, :]
    for k in range(NREG):
      v = buf[k, j, rows, :].astype(jnp.float32)
      buf[k, j, rows, :] = (v * sc).astype(buf.dtype)
    idx = (slice(None), j, rows, slice(None))
    pltpu.make_async_copy(buf.at[idx], o_hbm.at[idx], sem.at[0]).start()

  def first_row(cb, carry):
    scale_and_send(0, cb)
    return carry

  for cb in range(F):
    gate(cb)
  lax.fori_loop(0, F, first_row, 0)
  for cb in range(F, NCB):
    gate(cb)
  lax.fori_loop(F, NCB, first_row, 0)

  def write_body(j, carry):
    for cb in range(NCB):
      scale_and_send(j, cb)
    return carry

  lax.fori_loop(1, J, write_body, 0)
  pltpu.make_async_copy(buf, o_hbm, sem.at[0]).wait()


@jax.jit
def pallas_standalone__channel_attn_cbam__vision_kernel(
    x: jax.Array,
    w1: jax.Array,
    w2: jax.Array,
):
  B, H, W, C = x.shape
  R = w1.shape[1]
  assert B == 1 and H % NREG == 0
  shape = (NREG, H // NREG, C, W)
  out = pl.pallas_call(
      _cbam_kernel,
      in_specs=[pl.BlockSpec(memory_space=pl.ANY)] * 3,
      out_specs=pl.BlockSpec(memory_space=pl.ANY),
      out_shape=jax.ShapeDtypeStruct(shape, x.dtype),
      scratch_shapes=[
          pltpu.VMEM(shape, x.dtype),
          pltpu.VMEM((R, C), w1.dtype),
          pltpu.VMEM((R, C), w2.dtype),
          pltpu.VMEM((C, R), jnp.float32),
          pltpu.VMEM((C, R), jnp.float32),
          pltpu.VMEM((C, W), jnp.float32),
          pltpu.VMEM((C, W), jnp.float32),
          pltpu.VMEM((C, W), jnp.float32),
          pltpu.SemaphoreType.DMA((NS,)),
      ],
      compiler_params=pltpu.CompilerParams(vmem_limit_bytes=64 * 1024 * 1024),
  )(x.transpose(0, 1, 3, 2).reshape(shape), w1.T, w2)
  return out.reshape(B, H, C, W).transpose(0, 1, 3, 2)
```
